```python
import os as _os
_os.environ.setdefault('JAX_PLATFORMS', 'cpu')
import jax
import jax.numpy as jnp

def _softmax(x, axis=-1):
    return jax.nn.softmax(x, axis=axis)

def _gelu(x):
    return jax.nn.gelu(x, approximate=True)

def _silu(x):
    return jax.nn.silu(x)

def _sigmoid(x):
    return jax.nn.sigmoid(x)

def _layernorm(x, axis=-1, eps=1e-05):
    m = jnp.mean(x, axis=axis, keepdims=True)
    v = jnp.var(x, axis=axis, keepdims=True)
    return (x - m) / jnp.sqrt(v + eps)

def _scatter_add(tgt, idx, src, axis=0):
    return tgt.at[idx].add(src)

def _segment_sum(src, seg, n):
    return jax.ops.segment_sum(src, seg, n)

class _Rng:

    def __init__(self, key):
        self._k = key

    def _next(self):
        self._k, sub = jax.random.split(self._k)
        return sub

    def normal(self, shape):
        return jax.random.normal(self._next(), shape, dtype=jnp.bfloat16)

    def randint(self, lo, hi, shape):
        return jax.random.randint(self._next(), shape, lo, hi, dtype=jnp.int32)

    def uniform(self, shape, lo=0.0, hi=1.0):
        return jax.random.uniform(self._next(), shape, jnp.bfloat16, lo, hi)

    def permutation(self, n):
        return jax.random.permutation(self._next(), n)
kernel_name = 'standalone__autoregressive_conv_wavenet__speech'

def setup_inputs():
    _rng = _Rng(jax.random.key(int.from_bytes(__import__("os").urandom(4), "little")))
    _w = lambda a: (lambda t: t.astype(jnp.bfloat16) if jnp.issubdtype(t.dtype, jnp.floating) else t)(jnp.asarray(a))
    B, T, D, K = (2, 4000, 512, 31)
    return {'x': _w((lambda *s: _rng.normal(s) * 0.05)(B, T, D)), 'w': _w((lambda *s: _rng.normal(s) * 0.05)(K, D, 2 * D)), 'w_o': _w((lambda *s: _rng.normal(s) * 0.05)(D, D))}

def reference(x, w, w_o):
    B, T, D = x.shape
    K = w.shape[0]
    dil = 2
    pad = (K - 1) * dil
    xp = jnp.pad(x, ((0, 0), (pad, 0), (0, 0)))
    h = jnp.einsum('btc,cd->btd', xp[:, pad:pad + T, :], w[0])
    for i in range(1, K):
        off = pad - i * dil
        h = h + jnp.einsum('btc,cd->btd', xp[:, off:off + T, :], w[i])
    f = h[..., :D].copy()
    g = h[..., D:].copy()
    z = jnp.tanh(f) * _sigmoid(g)
    return z @ w_o
```

```python
import functools

import jax
import jax.numpy as jnp
import jax.experimental.pallas as pl
import jax.experimental.pallas.tpu as pltpu


def _wavenet_kernel(x_ref, halo_ref, w_ref, wo_ref, o_ref, xwin_ref, acc_ref, *, TT, H, K, dil):
    t = pl.program_id(1)
    D = x_ref.shape[-1]
    halo = halo_ref[0]
    xwin_ref[0:H, :] = jnp.where(t > 0, halo, jnp.zeros_like(halo))
    xwin_ref[H:H + TT, :] = x_ref[0]

    for i in range(K):
        off = H - i * dil
        contrib = jnp.dot(xwin_ref[off:off + TT, :], w_ref[i], preferred_element_type=jnp.float32)
        if i == 0:
            acc_ref[...] = contrib
        else:
            acc_ref[...] += contrib

    h = acc_ref[...]
    f = h[:, :D]
    g = h[:, D:]
    z = jnp.tanh(f) * jax.nn.sigmoid(g)
    o_ref[0] = jnp.dot(z.astype(jnp.bfloat16), wo_ref[...], preferred_element_type=jnp.float32).astype(o_ref.dtype)


@jax.jit
def pallas_standalone__autoregressive_conv_wavenet__speech_kernel(
    x: jax.Array,
    w: jax.Array,
    w_o: jax.Array,
):
    B, T, D = x.shape
    K = w.shape[0]
    dil = 2
    TT = 400
    H = 80
    assert T % TT == 0 and TT % H == 0 and H >= (K - 1) * dil
    r = TT // H

    kernel = functools.partial(_wavenet_kernel, TT=TT, H=H, K=K, dil=dil)
    return pl.pallas_call(
        kernel,
        grid=(B, T // TT),
        in_specs=[
            pl.BlockSpec((1, TT, D), lambda b, t: (b, t, 0)),
            pl.BlockSpec((1, H, D), lambda b, t: (b, jnp.maximum(t * r - 1, 0), 0)),
            pl.BlockSpec((K, D, 2 * D), lambda b, t: (0, 0, 0), pipeline_mode=pl.Buffered(1)),
            pl.BlockSpec((D, D), lambda b, t: (0, 0), pipeline_mode=pl.Buffered(1)),
        ],
        out_specs=pl.BlockSpec((1, TT, D), lambda b, t: (b, t, 0)),
        out_shape=jax.ShapeDtypeStruct((B, T, D), x.dtype),
        scratch_shapes=[
            pltpu.VMEM((H + TT, D), x.dtype),
            pltpu.VMEM((TT, 2 * D), jnp.float32),
        ],
        compiler_params=pltpu.CompilerParams(
            dimension_semantics=("arbitrary", "arbitrary"),
            vmem_limit_bytes=100 * 1024 * 1024,
        ),
    )(x, x, w, w_o)
```

```python
import functools

import jax
import jax.numpy as jnp
from jax import lax
import jax.experimental.pallas as pl
import jax.experimental.pallas.tpu as pltpu


def _wavenet_kernel(x_ref, halo_ref, w_hbm, wo_hbm, o_ref, xwin_ref, w_vmem, wo_vmem, z_ref, acc_ref, sems,
                    *, TT, H, K, dil, CW):
    b = pl.program_id(0)
    t = pl.program_id(1)
    D = x_ref.shape[-1]
    nchunks = D // CW
    first = jnp.logical_and(b == 0, t == 0)

    def w_copy(p, half):
        return pltpu.make_async_copy(
            w_hbm.at[:, :, pl.ds(pl.multiple_of(half * D + p * CW, CW), CW)],
            w_vmem.at[p, :, :, pl.ds(half * CW, CW)],
            sems.at[2 * p + half])

    def wo_copy():
        return pltpu.make_async_copy(wo_hbm, wo_vmem, sems.at[2 * nchunks])

    @pl.when(first)
    def _():
        for p in range(nchunks):
            w_copy(p, 0).start()
            w_copy(p, 1).start()
        wo_copy().start()

    halo = halo_ref[0]
    xwin_ref[0:H, :] = jnp.where(t > 0, halo, jnp.zeros_like(halo))
    xwin_ref[H:H + TT, :] = x_ref[0]

    def chunk_body(p, carry):
        @pl.when(first)
        def _():
            w_copy(p, 0).wait()
            w_copy(p, 1).wait()

        for i in range(K):
            off = H - i * dil
            contrib = jnp.dot(xwin_ref[off:off + TT, :], w_vmem[p, i], preferred_element_type=jnp.float32)
            if i == 0:
                acc_ref[...] = contrib
            elif i < K - 1:
                acc_ref[...] += contrib
            else:
                h = acc_ref[...] + contrib
        z = jnp.tanh(h[:, :CW]) * jax.nn.sigmoid(h[:, CW:])
        z_ref[:, pl.ds(pl.multiple_of(p * CW, CW), CW)] = z.astype(z_ref.dtype)
        return carry

    lax.fori_loop(0, nchunks, chunk_body, 0)

    @pl.when(first)
    def _():
        wo_copy().wait()

    o_ref[0] = jnp.dot(z_ref[...], wo_vmem[...], preferred_element_type=jnp.float32).astype(o_ref.dtype)


@jax.jit
def pallas_standalone__autoregressive_conv_wavenet__speech_kernel(
    x: jax.Array,
    w: jax.Array,
    w_o: jax.Array,
):
    B, T, D = x.shape
    K = w.shape[0]
    dil = 2
    TT = 800
    H = 80
    CW = 128
    assert T % TT == 0 and TT % H == 0 and H >= (K - 1) * dil
    r = TT // H
    nchunks = D // CW

    kernel = functools.partial(_wavenet_kernel, TT=TT, H=H, K=K, dil=dil, CW=CW)
    return pl.pallas_call(
        kernel,
        grid=(B, T // TT),
        in_specs=[
            pl.BlockSpec((1, TT, D), lambda b, t: (b, t, 0)),
            pl.BlockSpec((1, H, D), lambda b, t: (b, jnp.maximum(t * r - 1, 0), 0)),
            pl.BlockSpec(memory_space=pl.ANY),
            pl.BlockSpec(memory_space=pl.ANY),
        ],
        out_specs=pl.BlockSpec((1, TT, D), lambda b, t: (b, t, 0)),
        out_shape=jax.ShapeDtypeStruct((B, T, D), x.dtype),
        scratch_shapes=[
            pltpu.VMEM((H + TT, D), x.dtype),
            pltpu.VMEM((nchunks, K, D, 2 * CW), w.dtype),
            pltpu.VMEM((D, D), w_o.dtype),
            pltpu.VMEM((TT, D), jnp.bfloat16),
            pltpu.VMEM((TT, 2 * CW), jnp.float32),
            pltpu.SemaphoreType.DMA((2 * nchunks + 1,)),
        ],
        compiler_params=pltpu.CompilerParams(
            dimension_semantics=("arbitrary", "arbitrary"),
            vmem_limit_bytes=100 * 1024 * 1024,
        ),
    )(x, x, w, w_o)
```
